```python
import jax
import jax.numpy as jnp

def _softmax(x, axis=-1):
    return jax.nn.softmax(x, axis=axis)
def _gelu(x):
    return jax.nn.gelu(x, approximate=True)
def _silu(x):
    return jax.nn.silu(x)
def _sigmoid(x):
    return jax.nn.sigmoid(x)
def _layernorm(x, axis=-1, eps=1e-5):
    m = jnp.mean(x, axis=axis, keepdims=True)
    v = jnp.var(x, axis=axis, keepdims=True)
    return (x - m) / jnp.sqrt(v + eps)
def _scatter_add(tgt, idx, src, axis=0):
    return tgt.at[idx].add(src)
def _segment_sum(src, seg, n):
    return jax.ops.segment_sum(src, seg, n)
class _Rng:
    def __init__(self, key):
        self._k = key
    def _next(self):
        self._k, sub = jax.random.split(self._k)
        return sub
    def normal(self, shape):
        return jax.random.normal(self._next(), shape, dtype=jnp.bfloat16)
    def randint(self, lo, hi, shape):
        return jax.random.randint(self._next(), shape, lo, hi, dtype=jnp.int32)
    def uniform(self, shape, lo=0.0, hi=1.0):
        return jax.random.uniform(self._next(), shape, jnp.bfloat16, lo, hi)
    def permutation(self, n):
        return jax.random.permutation(self._next(), n)


kernel_name = 'standalone__structured_sparse_n_m__ragged'

def setup_inputs():
    _rng = _Rng(jax.random.key(int.from_bytes(__import__("os").urandom(4), "little")))
    _w = (lambda a: (lambda t: t.astype(jnp.bfloat16) if jnp.issubdtype(t.dtype, jnp.floating) else t)(jnp.asarray(a)))
    B, S, D = 16, 4096, 576
    assert D % 4 == 0, "d_model must be divisible by M=4 for 2:4 sparsity"
    return {
        "x": _w((lambda *s: _rng.normal(s) * 0.05)(B, S, D)),
        "w": _w((lambda *s: _rng.normal(s) * 0.05)(D, D)),
        "b": _w((lambda *s: _rng.normal(s) * 0.05)(D)),
    }

def reference(x, w, b):
    B, S, D = x.shape
    N, M = 2, 4
    G = D // M
    wg = w.reshape(G, M, D)
    mag = jnp.abs(wg)
    order = jnp.argsort(mag, 1)
    thr = jnp.take_along_axis(mag, order[:, M - N:M - N + 1, :], 1)
    mask = (lambda x, dt: x.astype(dt))(mag >= thr, w.dtype)
    wp = (wg * mask).reshape(D, D)
    return jnp.einsum("bsd,df->bsf", x, wp) + b
```

```python
import jax
import jax.numpy as jnp
import jax.experimental.pallas as pl
import jax.experimental.pallas.tpu as pltpu

_TS = 2048


def _prune(w):
    wf = w.astype(jnp.float32)
    mag = jnp.abs(wf)
    d = w.shape[0]
    row = jax.lax.broadcasted_iota(jnp.int32, wf.shape, 0)

    def partner(v, k):
        up = pltpu.roll(v, k, 0)
        dn = pltpu.roll(v, d - k, 0)
        return jnp.where((row & k) != 0, up, dn)

    p1 = partner(mag, 1)
    hi = jnp.maximum(mag, p1)
    lo = jnp.minimum(mag, p1)
    thr = jnp.maximum(jnp.minimum(hi, partner(hi, 2)), jnp.maximum(lo, partner(lo, 2)))
    return jnp.where(mag >= thr, wf, 0.0)


def _kernel(x_ref, w_ref, b_ref, o_ref, wt_ref):
    @pl.when(jnp.logical_and(pl.program_id(0) == 0, pl.program_id(1) == 0))
    def _():
        wt_ref[...] = _prune(w_ref[...]).T.astype(jnp.bfloat16)

    acc = jnp.dot(wt_ref[...], x_ref[...], preferred_element_type=jnp.float32)
    o_ref[...] = (acc + b_ref[...]).astype(o_ref.dtype)


@jax.jit
def pallas_standalone__structured_sparse_n_m__ragged_kernel(
    x: jax.Array,
    w: jax.Array,
    b: jax.Array,
):
    B, S, D = x.shape
    xt = jnp.transpose(x, (0, 2, 1))
    bc = b.reshape(D, 1)
    out = pl.pallas_call(
        _kernel,
        grid=(B, S // _TS),
        in_specs=[
            pl.BlockSpec((None, D, _TS), lambda i, j: (i, 0, j)),
            pl.BlockSpec((D, D), lambda i, j: (0, 0)),
            pl.BlockSpec((D, 1), lambda i, j: (0, 0)),
        ],
        out_specs=pl.BlockSpec((None, D, _TS), lambda i, j: (i, 0, j)),
        out_shape=jax.ShapeDtypeStruct((B, D, S), x.dtype),
        scratch_shapes=[pltpu.VMEM((D, D), jnp.bfloat16)],
        compiler_params=pltpu.CompilerParams(
            dimension_semantics=("arbitrary", "arbitrary"),
            vmem_limit_bytes=64 * 1024 * 1024,
        ),
    )(xt, w, bc)
    return jnp.transpose(out, (0, 2, 1))
```

```python
import jax
import jax.numpy as jnp
import jax.experimental.pallas as pl
import jax.experimental.pallas.tpu as pltpu

_C = 512
_NS = 4
_NU = 16
_KP = 64


def _prune_packed(w):
    R, D = w.shape
    wu = pltpu.bitcast(w, jnp.int32).reshape(R // 16, 8, D)
    a = pltpu.bitcast((wu << 16) & jnp.int32(0x7FFFFFFF), jnp.float32)
    b = pltpu.bitcast(wu & jnp.int32(0x7FFF0000), jnp.float32)
    hi = jnp.maximum(a, b)
    lo = jnp.minimum(a, b)
    t = jnp.maximum(jnp.minimum(hi, pltpu.roll(hi, 7, 1)), jnp.maximum(lo, pltpu.roll(lo, 7, 1)))
    sub = jax.lax.broadcasted_iota(jnp.int32, t.shape, 1)
    thr = jnp.where((sub & 1) == 0, t, pltpu.roll(t, 1, 1))
    m = jnp.where(a >= thr, jnp.int32(0xFFFF), 0) | jnp.where(b >= thr, jnp.int32(-65536), 0)
    return pltpu.bitcast((wu & m).reshape(R // 2, D), jnp.bfloat16)


def _kernel(x_hbm, w_hbm, b_hbm, o_hbm, xbuf, obuf, wbuf, bbuf, wt, isem, osem, wsem):
    B, D, S = x_hbm.shape
    C, NS, NU, KP = _C, _NS, _NU, _KP
    cpb = S // C
    nit = B * cpb // NU

    def pos(i, u):
        return i * (NU // cpb) + u // cpb, (u % cpb) * C

    def x_copy(i, u):
        s = u % NS
        bb, col = pos(i + u // NU, u % NU)
        return pltpu.make_async_copy(x_hbm.at[bb, :, pl.ds(col, C)], xbuf.at[s], isem.at[s])

    def o_copy(i, u):
        s = u % NS
        bb, col = pos(i + u // NU, u % NU)
        return pltpu.make_async_copy(obuf.at[s], o_hbm.at[bb, :, pl.ds(col, C)], osem.at[s])

    wcp = pltpu.make_async_copy(w_hbm, wbuf, wsem.at[0])
    bcp = pltpu.make_async_copy(b_hbm, bbuf, wsem.at[1])
    wcp.start()
    bcp.start()
    x_copy(0, 0).start()
    wcp.wait()
    bcp.wait()
    for s in range(1, NS):
        x_copy(0, s).start()

    wp = _prune_packed(wbuf[...])
    r = jax.lax.broadcasted_iota(jnp.int32, (KP, D), 0)
    brow = jnp.where(r == 0, bbuf[...].astype(jnp.float32)[None, :], 0.0).astype(jnp.bfloat16)
    wt[...] = jnp.concatenate([wp, brow], axis=0).T

    def body(i, carry):
        for u in range(NU):
            s = u % NS
            x_copy(i, u).wait()
            if u >= NS:
                o_copy(i, u - NS).wait()
            else:
                @pl.when(i > 0)
                def _():
                    o_copy(i, u - NS).wait()
            r = jax.lax.broadcasted_iota(jnp.int32, (KP, C), 0)
            ones = jnp.where(r == 0, 1.0, 0.0).astype(jnp.bfloat16)
            xa = jnp.concatenate([xbuf[s], ones], axis=0)
            acc = jnp.dot(wt[...], xa, preferred_element_type=jnp.float32)
            obuf[s] = acc.astype(jnp.bfloat16)
            o_copy(i, u).start()
            if u + NS < NU:
                x_copy(i, u + NS).start()
            else:
                @pl.when(i + 1 < nit)
                def _():
                    x_copy(i, u + NS).start()
        return carry

    jax.lax.fori_loop(0, nit, body, 0)
    for u in range(NU - NS, NU):
        o_copy(nit - 1, u).wait()


@jax.jit
def pallas_standalone__structured_sparse_n_m__ragged_kernel(
    x: jax.Array,
    w: jax.Array,
    b: jax.Array,
):
    B, S, D = x.shape
    assert D % 64 == 0 and S % _C == 0 and _NU % (S // _C) == 0 and (B * S // _C) % _NU == 0
    xt = jnp.transpose(x, (0, 2, 1))
    out = pl.pallas_call(
        _kernel,
        in_specs=[pl.BlockSpec(memory_space=pl.ANY)] * 3,
        out_specs=pl.BlockSpec(memory_space=pl.ANY),
        out_shape=jax.ShapeDtypeStruct((B, D, S), x.dtype),
        scratch_shapes=[
            pltpu.VMEM((_NS, D, _C), jnp.bfloat16),
            pltpu.VMEM((_NS, D, _C), jnp.bfloat16),
            pltpu.VMEM((D, D), jnp.bfloat16),
            pltpu.VMEM((D,), jnp.bfloat16),
            pltpu.VMEM((D, D + _KP), jnp.bfloat16),
            pltpu.SemaphoreType.DMA((_NS,)),
            pltpu.SemaphoreType.DMA((_NS,)),
            pltpu.SemaphoreType.DMA((2,)),
        ],
        compiler_params=pltpu.CompilerParams(
            vmem_limit_bytes=64 * 1024 * 1024,
            flags={"XLA_TPU_RESCHEDULE_DMA_DONES": True},
        ),
    )(xt, w, b)
    return jnp.transpose(out, (0, 2, 1))
```

```python
import jax
import jax.numpy as jnp
import jax.experimental.pallas as pl
import jax.experimental.pallas.tpu as pltpu

_C = 512
_NS = 3
_NU = 21
_MXU = 128
_TAIL = 9
_DMA = pltpu.SemaphoreType.DMA


def _prune(w):
    rows, cols = w.shape
    wu = pltpu.bitcast(w, jnp.int32).reshape(rows // 16, 8, cols)
    a = pltpu.bitcast((wu << 16) & jnp.int32(0x7FFFFFFF), jnp.float32)
    b = pltpu.bitcast(wu & jnp.int32(0x7FFF0000), jnp.float32)
    hi = jnp.maximum(a, b)
    lo = jnp.minimum(a, b)
    t = jnp.maximum(jnp.minimum(hi, pltpu.roll(hi, 7, 1)), jnp.maximum(lo, pltpu.roll(lo, 7, 1)))
    sub = jax.lax.broadcasted_iota(jnp.int32, t.shape, 1)
    thr = jnp.where((sub & 1) == 0, t, pltpu.roll(t, 1, 1))
    keep = jnp.where(a >= thr, jnp.int32(0xFFFF), 0) | jnp.where(b >= thr, jnp.int32(-65536), 0)
    return pltpu.bitcast((wu & keep).reshape(rows // 2, cols), jnp.bfloat16)


def _kernel(x_hbm, w_hbm, b_hbm, o_hbm, xbuf, obuf, wbuf, bbuf, wt, isem, osem, hsem):
    B, D, S = x_hbm.shape
    C, NS, NU = _C, _NS, _NU
    KP = wt.shape[1] - D
    per_batch = S // C
    n = B * per_batch
    nit = (n - 2) // NU
    ktiles = [(k, min(k + _MXU, D)) for k in range(0, D, _MXU)]
    last_k = len(ktiles) - 1

    def pos(c):
        if isinstance(c, int):
            return c // per_batch, (c % per_batch) * C
        return c // per_batch, pl.multiple_of((c % per_batch) * C, C)

    def x_copy(c, s):
        bb, col = pos(c)
        return pltpu.make_async_copy(x_hbm.at[bb, :, pl.ds(col, C)], xbuf[s], isem[s])

    def o_copy(c, s):
        bb, col = pos(c)
        return pltpu.make_async_copy(obuf[s], o_hbm.at[bb, :, pl.ds(col, C)], osem[s])

    def ones_rows():
        r = jax.lax.broadcasted_iota(jnp.int32, (KP, C), 0)
        return jnp.where(r == 0, 1.0, 0.0).astype(jnp.bfloat16)

    def x_aug(s):
        return jnp.concatenate([xbuf[s][...], ones_rows()], axis=0)

    def matmul(s):
        xv = x_aug(s)
        for m in range(0, C, _MXU):
            acc = jnp.dot(wt[...], xv[:, m:m + _MXU], preferred_element_type=jnp.float32)
            obuf[s][:, m:m + _MXU] = acc.astype(jnp.bfloat16)

    korder = [last_k] + list(range(last_k))
    pool = iter([hsem.at[i] for i in range(hsem.shape[0])] + [isem[0]] + list(osem))
    b_copy = pltpu.make_async_copy(b_hbm, bbuf, next(pool))
    b_copy.start()
    w_piece, x_piece = {}, {}
    for j in korder:
        k0, k1 = ktiles[j]
        rows = pl.ds(k0, k1 - k0)
        w_piece[j] = pltpu.make_async_copy(w_hbm.at[rows], wbuf.at[rows], next(pool))
        x_piece[j] = pltpu.make_async_copy(x_hbm.at[0, rows, pl.ds(0, C)], xbuf[0].at[rows], next(pool))
        w_piece[j].start()
        x_piece[j].start()
    for c in range(1, NS):
        x_copy(c, c).start()

    acc = None
    for j in korder:
        k0, k1 = ktiles[j]
        w_piece[j].wait()
        wp = _prune(wbuf[k0:k1, :])
        if j == last_k:
            b_copy.wait()
            r = jax.lax.broadcasted_iota(jnp.int32, (KP, D), 0)
            bias = jnp.where(r == 0, bbuf[...].astype(jnp.float32)[None, :], 0.0)
            wp = jnp.concatenate([wp, bias.astype(jnp.bfloat16)], axis=0)
        wtj = wp.T
        wt[:, k0:k0 + wtj.shape[1]] = wtj
        x_piece[j].wait()
        xj = xbuf[0][k0:k1, :]
        if j == last_k:
            xj = jnp.concatenate([xj, ones_rows()], axis=0)
        part = jnp.dot(wtj, xj, preferred_element_type=jnp.float32)
        acc = part if acc is None else acc + part
    obuf[0][...] = acc.astype(jnp.bfloat16)
    o_copy(0, 0).start()
    x_copy(NS, 0).start()

    def body(i, carry):
        for u in range(NU):
            c = 1 + i * NU + u
            s = (1 + u) % NS
            x_copy(c, s).wait()
            if 1 + u >= NS:
                o_copy(c - NS, s).wait()
            else:
                @pl.when(i > 0)
                def _():
                    o_copy(c - NS, s).wait()
            matmul(s)
            o_copy(c, s).start()
            if 1 + (nit - 1) * NU + u + NS < n:
                x_copy(c + NS, s).start()
            else:
                @pl.when(i + 1 < nit)
                def _():
                    x_copy(c + NS, s).start()
        return carry

    jax.lax.fori_loop(0, nit, body, 0)

    c = n - 1
    s = c % NS
    x_copy(c, s).wait()
    o_copy(c - NS, s).wait()
    bb, col = pos(c)
    slab = D // _TAIL
    xv = x_aug(s)
    slabs = []
    for p in range(_TAIL):
        rows = pl.ds(p * slab, slab)
        acc = jnp.dot(wt[p * slab:(p + 1) * slab, :], xv, preferred_element_type=jnp.float32)
        obuf[s][p * slab:(p + 1) * slab, :] = acc.astype(jnp.bfloat16)
        cp = pltpu.make_async_copy(obuf[s].at[rows], o_hbm.at[bb, rows, pl.ds(col, C)], hsem.at[0])
        cp.start()
        slabs.append(cp)
    for cc in range(n - NS, n - 1):
        o_copy(cc, cc % NS).wait()
    for cp in slabs:
        cp.wait()


@jax.jit
def pallas_standalone__structured_sparse_n_m__ragged_kernel(
    x: jax.Array,
    w: jax.Array,
    b: jax.Array,
):
    B, S, D = x.shape
    nk = pl.cdiv(D, _MXU)
    kp = nk * _MXU - D if D % _MXU else _MXU
    assert S % _C == 0 and (B * S // _C - 2) % _NU == 0 and _NU % _NS == 0
    assert D % 64 == 0 and D % (16 * _TAIL) == 0 and D > _MXU
    n_head = 2 * nk + 1 - (1 + _NS)
    xt = jnp.transpose(x, (0, 2, 1))
    out = pl.pallas_call(
        _kernel,
        in_specs=[pl.BlockSpec(memory_space=pl.ANY)] * 3,
        out_specs=pl.BlockSpec(memory_space=pl.ANY),
        out_shape=jax.ShapeDtypeStruct((B, D, S), x.dtype),
        scratch_shapes=[
            [pltpu.VMEM((D, _C), jnp.bfloat16) for _ in range(_NS)],
            [pltpu.VMEM((D, _C), jnp.bfloat16) for _ in range(_NS)],
            pltpu.VMEM((D, D), jnp.bfloat16),
            pltpu.VMEM((D,), jnp.bfloat16),
            pltpu.VMEM((D, D + kp), jnp.bfloat16),
            [_DMA(()) for _ in range(_NS)],
            [_DMA(()) for _ in range(_NS)],
            _DMA((n_head,)),
        ],
        compiler_params=pltpu.CompilerParams(
            vmem_limit_bytes=64 * 1024 * 1024,
            flags={"XLA_TPU_RESCHEDULE_DMA_DONES": True},
        ),
    )(xt, w, b)
    return jnp.transpose(out, (0, 2, 1))
```
